```python
import os as _os
_os.environ.setdefault('JAX_PLATFORMS', 'cpu')
import jax
import jax.numpy as jnp

def _softmax(x, axis=-1):
    return jax.nn.softmax(x, axis=axis)

def _gelu(x):
    return jax.nn.gelu(x, approximate=True)

def _silu(x):
    return jax.nn.silu(x)

def _sigmoid(x):
    return jax.nn.sigmoid(x)

def _layernorm(x, axis=-1, eps=1e-05):
    m = jnp.mean(x, axis=axis, keepdims=True)
    v = jnp.var(x, axis=axis, keepdims=True)
    return (x - m) / jnp.sqrt(v + eps)

def _scatter_add(tgt, idx, src, axis=0):
    return tgt.at[idx].add(src)

def _segment_sum(src, seg, n):
    return jax.ops.segment_sum(src, seg, n)

class _Rng:

    def __init__(self, key):
        self._k = key

    def _next(self):
        self._k, sub = jax.random.split(self._k)
        return sub

    def normal(self, shape):
        return jax.random.normal(self._next(), shape, dtype=jnp.bfloat16)

    def randint(self, lo, hi, shape):
        return jax.random.randint(self._next(), shape, lo, hi, dtype=jnp.int32)

    def uniform(self, shape, lo=0.0, hi=1.0):
        return jax.random.uniform(self._next(), shape, jnp.bfloat16, lo, hi)

    def permutation(self, n):
        return jax.random.permutation(self._next(), n)
kernel_name = 'adaLN_cond__sliding_local_dilated__dense_activation_relu__prompt'

def setup_inputs():
    _rng = _Rng(jax.random.key(int.from_bytes(__import__("os").urandom(4), "little")))
    _w = lambda a: (lambda t: t.astype(jnp.bfloat16) if jnp.issubdtype(t.dtype, jnp.floating) else t)(jnp.asarray(a))

    def _A_setup():
        B, S, D = (1, 2048, 576)
        return {'x': _w((lambda *s: _rng.normal(s) * 0.05)(B, S, D)), 'wqkv': _w((lambda *s: _rng.normal(s) * 0.05)(D, 3 * D)), 'wo': _w((lambda *s: _rng.normal(s) * 0.05)(D, D))}
    _A_in = _A_setup()

    def _B_setup():
        B, S, D, Dff = (1, 2048, 576, 4608)
        return {'x': _w((lambda *s: _rng.normal(s) * 0.05)(B, S, D)), 'w1': _w((lambda *s: _rng.normal(s) * 0.05)(D, Dff)), 'w2': _w((lambda *s: _rng.normal(s) * 0.05)(Dff, D))}
    _B_in = _B_setup()
    return {'A_x': _A_in['x'], 'A_wqkv': _A_in['wqkv'], 'A_wo': _A_in['wo'], 'B_x': _B_in['x'], 'B_w1': _B_in['w1'], 'B_w2': _B_in['w2'], 'c': _w((lambda *s: _rng.normal(s) * 0.05)(1, 576) * 8.0), 'w_mod': _w((lambda *s: _rng.normal(s) * 0.05)(576, 6 * 576) * 576 ** (-0.5) * 8.0)}

def reference(A_x, A_wqkv, A_wo, B_x, B_w1, B_w2, c, w_mod):

    def _A_ref(x, wqkv, wo):
        B, S, D = x.shape
        H = 32
        Dh = D // H
        W, dil = (8, 2)
        qkv = (lambda x, *d: x.transpose(*d))((x @ wqkv).reshape(B, S, 3, H, Dh), 2, 0, 3, 1, 4)
        q, k, v = (qkv[0], qkv[1], qkv[2])
        scale = Dh ** (-0.5)
        pos = jnp.arange(S)
        off = jnp.arange(W) * dil
        idx = pos[:, None] - off[None, :]
        mask = idx >= 0
        idx_c = jnp.where(mask, idx, 0).reshape(-1)
        kg = k[:, :, idx_c, :].reshape(B, H, S, W, Dh)
        vg = v[:, :, idx_c, :].reshape(B, H, S, W, Dh)
        logits = jnp.einsum('bhsd,bhswd->bhsw', q, kg) * scale
        logits = jnp.where(mask[None, None, :, :], logits, -1000000000.0)
        attn = _softmax(logits, axis=-1)
        o = jnp.einsum('bhsw,bhswd->bhsd', attn, vg)
        return (lambda x, *d: x.transpose(*d))(o, 0, 2, 1, 3).reshape(B, S, D) @ wo

    def _B_ref(x, w1, w2):
        h = jnp.einsum('bsd,df->bsf', x, w1)
        zero = jnp.zeros_like(h)
        h = jnp.maximum(h, zero)
        return jnp.einsum('bsf,fd->bsd', h, w2)
    x = A_x
    mod = (_silu(c) @ w_mod).reshape(c.shape[0], 6, 1, -1)
    sa, ca, ga, sb, cb, gb = (mod[:, 0].copy(), mod[:, 1].copy(), mod[:, 2].copy(), mod[:, 3].copy(), mod[:, 4].copy(), mod[:, 5].copy())
    h = _layernorm(x, axis=-1) * (1 + ca) + sa
    x = x + ga * _A_ref(h, A_wqkv, A_wo)
    h = _layernorm(x, axis=-1) * (1 + cb) + sb
    x = x + gb * _B_ref(h, B_w1, B_w2)
    return x
```

```python
import functools
import numpy as np
import jax
import jax.numpy as jnp
from jax import lax
import jax.experimental.pallas as pl
import jax.experimental.pallas.tpu as pltpu

S, D, H, DH, FF = 2048, 576, 32, 18, 4608
W, DIL = 8, 2
HALO = 16
TM = 512
NB = S // TM
RC = 16
EPS = 1e-5
F32, BF16 = jnp.float32, jnp.bfloat16
NN = (((1,), (0,)), ((), ()))
NT = (((1,), (1,)), ((), ()))
TN = (((0,), (0,)), ((), ()))


def _dg(a, b, dn):
    return lax.dot_general(a, b, dn, preferred_element_type=F32)


def _dest_row(t, d):
    if d < 16:
        return t * 512 + d * 32
    return 1536 + t * 64 + (d - 16) * 32


def kernel(xT_hbm, wqkv_hbm, wo_hbm, w1_hbm, w2T_hbm, c_hbm, wm_hbm, outT_hbm,
           xb, wqkv_v, wT32, wpT, wo_v, wo32, wopT, w1_v, w2T_v, wm_v, c_v, modT,
           q_s, k_s, v_s, o_s, x1T, h2T, outb, sems):
    def cp(src, dst, i):
        return pltpu.make_async_copy(src, dst, sems.at[i])

    dm_c = cp(c_hbm, c_v, 0)
    dm_wmA = cp(wm_hbm.at[:, pl.ds(0, 2 * D)], wm_v.at[:, pl.ds(0, 2 * D)], 1)
    dm_wmB = cp(wm_hbm.at[:, pl.ds(2 * D, 4 * D)], wm_v.at[:, pl.ds(2 * D, 4 * D)], 2)
    dm_wqkv = cp(wqkv_hbm, wqkv_v, 3)
    dm_wo = cp(wo_hbm, wo_v, 4)
    dm_w1 = cp(w1_hbm, w1_v, 5)
    dm_w2 = cp(w2T_hbm, w2T_v, 6)
    dm_x = [cp(xT_hbm.at[:, pl.ds(j * TM, TM)], xb.at[:, pl.ds(j * TM, TM)], 7 + j) for j in range(NB)]
    dm_out = [cp(outb.at[:, pl.ds(j * TM, TM)], outT_hbm.at[:, pl.ds(j * TM, TM)], 7 + NB + j) for j in range(NB)]

    dm_c.start(); dm_wmA.start(); dm_x[0].start(); dm_wqkv.start()

    zero_halo = jnp.zeros((HALO, 128), F32)
    for t in range(5):
        k_s[t, pl.ds(0, HALO), :] = zero_halo
        v_s[t, pl.ds(0, HALO), :] = zero_halo
    wT32[4] = jnp.zeros((3 * D, 128), F32)
    wo32[4] = jnp.zeros((D, 128), F32)

    def mod_part(lo, n):
        sc = c_v[...].astype(F32)
        sc = (sc * jax.nn.sigmoid(sc)).astype(BF16)
        sc = jnp.broadcast_to(sc, (16, D))
        m = _dg(sc, wm_v[:, lo:lo + n], NN)
        m = jnp.broadcast_to(m[0:1, :], (128, n))
        modT[pl.ds(lo, n), :] = m.T

    dm_c.wait(); dm_wmA.wait()
    mod_part(0, 2 * D)

    dm_wqkv.wait()
    dm_wmB.start()
    for j in range(1, NB):
        dm_x[j].start()
    dm_wo.start(); dm_w1.start(); dm_w2.start()

    wT = wqkv_v[...].T.astype(F32)
    for s in range(4):
        wT32[s] = wT[:, s * 128:(s + 1) * 128]
    wT32[4, :, 0:64] = wT[:, 512:576]
    for t in range(3):
        for d in range(DH):
            r = _dest_row(t, d)
            for s in range(5):
                blk = wT32[s, pl.ds(t * D + d, H, stride=DH), :].astype(BF16)
                if s < 4:
                    wpT[pl.ds(r, H), s * 128:(s + 1) * 128] = blk
                else:
                    wpT[pl.ds(r, H), 512:576] = blk[:, 0:64]

    lane = lax.broadcasted_iota(jnp.int32, (TM, 128), 1)
    lo_half = lane < 64

    def ln_mod(xf, sh_off, sc_off):
        mean = jnp.sum(xf, axis=0, keepdims=True) * (1.0 / D)
        xc = xf - mean
        var = jnp.sum(xc * xc, axis=0, keepdims=True) * (1.0 / D)
        r = lax.rsqrt(var + EPS)
        return xc * r * (1.0 + modT[pl.ds(sc_off, D), :]) + modT[pl.ds(sh_off, D), :]

    def stage_A(j):
        dm_x[j].wait()
        hs = []
        for cidx in range(TM // 128):
            xf = xb[:, pl.ds(j * TM + cidx * 128, 128)].astype(F32)
            hs.append(ln_mod(xf, 0, D).astype(BF16))
        hT = jnp.concatenate(hs, axis=1)
        qkv = _dg(hT.T, wpT[...], NT)
        rows = pl.ds(j * TM, TM)
        rows_h = pl.ds(HALO + j * TM, TM)
        for t in range(4):
            q_s[t, rows, :] = qkv[:, t * 128:(t + 1) * 128]
            k_s[t, rows_h, :] = qkv[:, 512 + t * 128:512 + (t + 1) * 128]
            v_s[t, rows_h, :] = qkv[:, 1024 + t * 128:1024 + (t + 1) * 128]
        qk_t = qkv[:, 1536:1664]
        q_s[4, rows, :] = jnp.where(lo_half, qk_t, 0.0)
        k_s[4, rows_h, :] = jnp.where(lo_half, pltpu.roll(qk_t, 64, 1), 0.0)
        vt = qkv[:, 1664:1728]
        v_s[4, rows_h, :] = jnp.concatenate([vt, jnp.zeros_like(vt)], axis=1)

    cexp = float(DH ** -0.5 * np.log2(np.e))

    def stage_B(j):
        for rc in range(TM // RC):
            r0 = j * TM + rc * RC
            q = [q_s[t, pl.ds(r0, RC), :] for t in range(5)]
            T = []
            for w in range(W):
                acc = None
                for t in range(5):
                    p = q[t] * k_s[t, pl.ds(HALO + r0 - DIL * w, RC), :]
                    acc = p if acc is None else acc + p
                acc = acc + pltpu.roll(acc, 64, 1)
                acc = acc + pltpu.roll(acc, 32, 1)
                if r0 < HALO and w > 0:
                    pos = r0 + lax.broadcasted_iota(jnp.int32, (RC, 128), 0)
                    acc = jnp.where(pos >= DIL * w, acc, -1e30)
                T.append(acc)
            m = T[0]
            for w in range(1, W):
                m = jnp.maximum(m, T[w])
            e = [jnp.exp2((T[w] - m) * cexp) for w in range(W)]
            l = e[0]
            for w in range(1, W):
                l = l + e[w]
            rinv = 1.0 / l
            for t in range(5):
                acc = None
                for w in range(W):
                    p = e[w] * v_s[t, pl.ds(HALO + r0 - DIL * w, RC), :]
                    acc = p if acc is None else acc + p
                ot = (acc * rinv).astype(BF16)
                if t < 4:
                    o_s[pl.ds(r0, RC), t * 128:(t + 1) * 128] = ot
                else:
                    o_s[pl.ds(r0, RC), 512:576] = ot[:, 0:64]

    def stage_C(j):
        at = _dg(wopT[...], o_s[pl.ds(j * TM, TM), :], NT)
        for cidx in range(TM // 128):
            cols = pl.ds(j * TM + cidx * 128, 128)
            x1 = xb[:, cols].astype(F32) + modT[pl.ds(2 * D, D), :] * at[:, cidx * 128:(cidx + 1) * 128]
            x1T[:, cols] = x1
            h2T[:, cols] = ln_mod(x1, 3 * D, 4 * D).astype(BF16)

    def stage_D(j):
        cols = pl.ds(j * TM, TM)
        a = jnp.maximum(_dg(h2T[:, cols], w1_v[...], TN), 0.0).astype(BF16)
        yT = _dg(w2T_v[...], a, NT)
        for cidx in range(TM // 128):
            cc = pl.ds(j * TM + cidx * 128, 128)
            res = x1T[:, cc] + modT[pl.ds(5 * D, D), :] * yT[:, cidx * 128:(cidx + 1) * 128]
            outb[:, cc] = res.astype(BF16)
        dm_out[j].start()

    stage_A(0)

    dm_wmB.wait()
    mod_part(2 * D, 4 * D)
    dm_wo.wait()
    wof = wo_v[...].astype(F32)
    for s in range(4):
        wo32[s] = wof[:, s * 128:(s + 1) * 128]
    wo32[4, :, 0:64] = wof[:, 512:576]
    for s in range(5):
        blk = jnp.concatenate([wo32[s, pl.ds(d, H, stride=DH), :] for d in range(DH)], axis=0)
        bt = blk.T.astype(BF16)
        if s < 4:
            wopT[pl.ds(s * 128, 128), :] = bt
        else:
            wopT[pl.ds(512, 64), :] = bt[0:64, :]

    stage_B(0); stage_A(1)
    for j in range(1, NB):
        stage_C(j - 1)
        stage_B(j)
        if j + 1 < NB:
            stage_A(j + 1)
    stage_C(NB - 1)
    dm_w1.wait(); dm_w2.wait()
    for j in range(NB):
        stage_D(j)
    for j in range(NB):
        dm_out[j].wait()


def _call(xT, wqkv, wo, w1, w2T, c, wm):
    hbm = pl.BlockSpec(memory_space=pltpu.HBM)
    scratch = [
        pltpu.VMEM((D, S), BF16),
        pltpu.VMEM((D, 3 * D), BF16),
        pltpu.VMEM((5, 3 * D, 128), F32),
        pltpu.VMEM((3 * D, D), BF16),
        pltpu.VMEM((D, D), BF16),
        pltpu.VMEM((5, D, 128), F32),
        pltpu.VMEM((D, D), BF16),
        pltpu.VMEM((D, FF), BF16),
        pltpu.VMEM((D, FF), BF16),
        pltpu.VMEM((D, 6 * D), BF16),
        pltpu.VMEM((1, D), BF16),
        pltpu.VMEM((6 * D, 128), F32),
        pltpu.VMEM((5, S, 128), F32),
        pltpu.VMEM((5, HALO + S, 128), F32),
        pltpu.VMEM((5, HALO + S, 128), F32),
        pltpu.VMEM((S, D), BF16),
        pltpu.VMEM((D, S), F32),
        pltpu.VMEM((D, S), BF16),
        pltpu.VMEM((D, S), BF16),
        pltpu.SemaphoreType.DMA((7 + 2 * NB,)),
    ]
    return pl.pallas_call(
        kernel,
        out_shape=jax.ShapeDtypeStruct((D, S), BF16),
        in_specs=[hbm] * 7,
        out_specs=hbm,
        scratch_shapes=scratch,
        compiler_params=pltpu.CompilerParams(vmem_limit_bytes=110 * 1024 * 1024),
    )(xT, wqkv, wo, w1, w2T, c, wm)


@jax.jit
def pallas_adaLN_cond__sliding_local_dilated__dense_activation_relu__prompt_kernel(A_x, A_wqkv, A_wo, B_x, B_w1, B_w2, c, w_mod):
    xT = A_x.reshape(S, D).T
    outT = _call(xT, A_wqkv, A_wo, B_w1, B_w2.T, c, w_mod)
    return outT.T.reshape(1, S, D)
```

```python
import contextlib
import numpy as np
import jax
import jax.numpy as jnp
from jax import lax
import jax.experimental.pallas as pl
import jax.experimental.pallas.tpu as pltpu

S, D, H, DH, FF = 2048, 576, 32, 18, 4608
W, DIL = 8, 2
HALO = 16
TM = 512
NB = S // TM
FC = 512
NF = FF // FC
EPS = 1e-5
F32, BF16 = jnp.float32, jnp.bfloat16
NN = (((1,), (0,)), ((), ()))
NT = (((1,), (1,)), ((), ()))
SCOPES = 0
LASTSPLIT = 2
FOLD = 1
BLOOP = 'o8'
ORDER = '0cGHIJXKYZmo12'
PROG = 'w0 S wcG g0 K0:3 wH g1 K0:012 K1:3 wI g2 K1:012 K2:3 wJ g3 K2:012 K3:3 wKX g4 K3:012 L1 K4:3012 wYZ A1:3012 L2 L3 wmo B0:b8 A2:3012 M A3:30 | C0 A3:12 w12 D0:0-8 B1:o8 | C1 D0:8-9 D1:0-8 B2:o8 | C2 D1:8-9 D2:0-8 B3:o8 o0 | C3 D2:8-9 o12 D3'


def _dg(a, b, dn):
    return lax.dot_general(a, b, dn, preferred_element_type=F32)


def _dest_row(t, d):
    if d < 16:
        return t * 512 + d * 32
    return 1536 + t * 64 + (d - 16) * 32


def kernel(xT_hbm, wqkv_hbm, wo_hbm, w1_hbm, w2T_hbm, c_hbm, wm_hbm, outT_hbm,
           wqkv_v, wT32, wpT, wo_v, wo32, wopT, w1_v, w2T_v, wm_v, c_v, modT,
           xb, hN, q_s, k_s, v_s, o_s, h2N, outb, tl_s, sems, rsem):

    def cp(src, dst, i):
        return pltpu.make_async_copy(src, dst, sems.at[i])

    def scope(name):
        return jax.named_scope(name) if SCOPES else contextlib.nullcontext()

    wq_cols = [(0, 640), (640, 512), (1152, 576)]
    dms = {
        "c": cp(c_hbm, c_v, 0),
        "m": cp(wm_hbm.at[:, pl.ds(2 * D, 4 * D)], wm_v.at[:, pl.ds(2 * D, 4 * D)], 2),
        "o": cp(wo_hbm, wo_v, 3), "1": cp(w1_hbm, w1_v, 4), "2": cp(w2T_hbm, w2T_v, 5),
    }
    KG = [(512, 64), (0, 128), (128, 128), (256, 128), (384, 128)]
    WMT = [[(4, 1), (8, 1)], [(0, 1), (5, 1)], [(1, 1), (6, 1)], [(2, 1), (7, 1)], [(3, 1)]]
    gdm = []
    si = 20
    for gi, (r0_, n_) in enumerate(KG):
        lst = [cp(wqkv_hbm.at[pl.ds(r0_, n_), :], wqkv_v.at[pl.ds(r0_, n_), :], si)]; si += 1
        for (t0, nt) in WMT[gi]:
            lst.append(cp(wm_hbm.at[:, pl.ds(t0 * 128, nt * 128)], wm_v.at[:, pl.ds(t0 * 128, nt * 128)], si)); si += 1
        gdm.append(lst)
    for j, ch in enumerate("0XYZ"):
        dms[ch] = cp(xT_hbm.at[:, pl.ds(j * TM, TM)], xb.at[j], 9 + j)

    def out_copy(j, lo, n, si):
        col0 = j * TM + lo
        if not isinstance(col0, int):
            col0 = pl.multiple_of(col0, 128)
        return cp(outb.at[j, :, pl.ds(lo, n)], outT_hbm.at[:, pl.ds(col0, n)], si)

    def mod_part(lo, n):
        sc = c_v[...].astype(F32)
        sc = (sc * jax.nn.sigmoid(sc)).astype(BF16)
        sc = jnp.broadcast_to(sc, (16, D))
        m = _dg(sc, wm_v[:, lo:lo + n], NN)
        col = lo + lax.broadcasted_iota(jnp.int32, (1, n), 1)
        is_scale = ((col >= D) & (col < 2 * D)) | ((col >= 4 * D) & (col < 5 * D))
        m = m[0:1, :] + jnp.where(is_scale, 1.0, 0.0)
        modT[pl.ds(lo, n), :] = jnp.broadcast_to(m, (128, n)).T

    def prep_slab(s):
        n_ = 128 if s < 4 else 64
        wT = wqkv_v[pl.ds(s * 128, n_), :].T.astype(F32)
        wT32[s] = wT if s < 4 else jnp.concatenate([wT, jnp.zeros((3 * D, 64), F32)], axis=1)
        for t in range(3):
            for d in range(DH):
                r = _dest_row(t, d)
                blk = wT32[s, pl.ds(t * D + d, H, stride=DH), :].astype(BF16)
                wpT[pl.ds(r, H), pl.ds(s * 128, n_)] = blk if s < 4 else blk[:, 0:64]

    def stats0():
        st = []
        for cidx in range(TM // 128):
            xf = xb[0, :, pl.ds(cidx * 128, 128)].astype(F32)
            mean = jnp.sum(xf, axis=0, keepdims=True) * (1.0 / D)
            xc = xf - mean
            var = jnp.sum(xc * xc, axis=0, keepdims=True) * (1.0 / D)
            st.append((mean, lax.rsqrt(var + EPS)))
        state["st0"] = st

    def group0(gi):
        for (t0, nt) in WMT[gi]:
            mod_part(t0 * 128, nt * 128)
        r0_, n_ = KG[gi]
        for s in range(r0_ // 128, (r0_ + n_ + 127) // 128):
            prep_slab(s)
        for cidx in range(TM // 128):
            mean, r = state["st0"][cidx]
            xf = xb[0, pl.ds(r0_, n_), pl.ds(cidx * 128, 128)].astype(F32)
            h = (xf - mean) * r * modT[pl.ds(D + r0_, n_), :] + modT[pl.ds(r0_, n_), :]
            hN[0, pl.ds(cidx * 128, 128), pl.ds(r0_, n_)] = h.astype(BF16).T

    def A0k(gi, g):
        r0_, n_ = KG[gi]
        hh = hN[0, :, pl.ds(r0_, n_)]
        if g < 3:
            r = _dg(hh, wpT[pl.ds(g * 512, 512), pl.ds(r0_, n_)], NT)
        else:
            r = _dg(wpT[pl.ds(1536, 192), pl.ds(r0_, n_)], hh, NT)
        last = gi == len(KG) - 1
        if g == 3:
            if gi > 0:
                r = r + tl_s[...]
            if last:
                A_store(0, 3, r)
            else:
                tl_s[...] = r
            return
        dst = [q_s, k_s, v_s][g]
        rows = pl.ds(0 if g == 0 else HALO, TM)
        vals = []
        for t in range(4):
            val = r[:, t * 128:(t + 1) * 128]
            if gi > 0:
                val = val + dst[0, t, rows, :]
            vals.append(val)
        if last:
            A_store(0, g, jnp.concatenate(vals, axis=1))
        else:
            for t in range(4):
                dst[0, t, rows, :] = vals[t]

    def prep_wo():
        wof = wo_v[...].astype(F32)
        for s in range(4):
            wo32[s] = wof[:, s * 128:(s + 1) * 128]
        wo32[4] = jnp.concatenate([wof[:, 512:576], jnp.zeros((D, 64), F32)], axis=1)
        for s in range(5):
            blk = jnp.concatenate([wo32[s, pl.ds(d, H, stride=DH), :] for d in range(DH)], axis=0)
            bt = blk.T.astype(BF16)
            if s < 4:
                wopT[pl.ds(s * 128, 128), :] = bt
            else:
                wopT[pl.ds(512, 64), :] = bt[0:64, :]

    def ln_mod(xf, sh_off, sc_off):
        mean = jnp.sum(xf, axis=0, keepdims=True) * (1.0 / D)
        xc = xf - mean
        var = jnp.sum(xc * xc, axis=0, keepdims=True) * (1.0 / D)
        r = lax.rsqrt(var + EPS)
        return xc * r * modT[pl.ds(sc_off, D), :] + modT[pl.ds(sh_off, D), :]

    def store_kv(dst, j, t, val):
        dst[j, t, pl.ds(HALO, TM), :] = val
        if j + 1 < NB:
            dst[j + 1, t, pl.ds(0, HALO), :] = val[TM - HALO:, :]

    def ln1(j):
        for cidx in range(TM // 128):
            xf = xb[j, :, pl.ds(cidx * 128, 128)].astype(F32)
            hN[j, pl.ds(cidx * 128, 128), :] = ln_mod(xf, 0, D).astype(BF16).T

    def A_store(j, g, r):
        if g < 3:
            for t in range(4):
                val = r[:, t * 128:(t + 1) * 128]
                if g == 0:
                    q_s[j, t] = val
                else:
                    store_kv(k_s if g == 1 else v_s, j, t, val)
            return
        lo_half = lax.broadcasted_iota(jnp.int32, (TM, 128), 1) < 64
        qk_t = r[0:128, :].T
        vt = r[128:192, :].T
        q_s[j, 4] = jnp.where(lo_half, qk_t, 0.0)
        store_kv(k_s, j, 4, jnp.where(lo_half, pltpu.roll(qk_t, 64, 1), 0.0))
        store_kv(v_s, j, 4, jnp.concatenate([vt, jnp.zeros_like(vt)], axis=1))

    def A(j, g):
        if g < 3:
            A_store(j, g, _dg(hN[j], wpT[pl.ds(g * 512, 512), :], NT))
        else:
            A_store(j, g, _dg(wpT[pl.ds(1536, 192), :], hN[j], NT))

    cexp = float(DH ** -0.5 * np.log2(np.e))

    def B(j, jo, var, first_block):
        kind, rc = var[0], int(var[1:])
        n = TM // rc

        def logits(r0, w, q):
            ps = [q[t] * k_s[j, t, pl.ds(HALO + r0 - DIL * w, rc), :] for t in range(5)]
            return ((ps[0] + ps[1]) + (ps[2] + ps[3])) + ps[4]

        def finish(r0, T):
            if first_block and r0 < HALO:
                pos = r0 + lax.broadcasted_iota(jnp.int32, (rc, 128), 0)
                T = [T[0]] + [jnp.where(pos >= DIL * w, T[w], -1e30) for w in range(1, W)]
            m = jnp.maximum(jnp.maximum(jnp.maximum(T[0], T[1]), jnp.maximum(T[2], T[3])),
                            jnp.maximum(jnp.maximum(T[4], T[5]), jnp.maximum(T[6], T[7])))
            e = [jnp.exp2((T[w] - m) * cexp) for w in range(W)]
            l = ((e[0] + e[1]) + (e[2] + e[3])) + ((e[4] + e[5]) + (e[6] + e[7]))
            rinv = 1.0 / l
            for t in range(5):
                p = [e[w] * v_s[j, t, pl.ds(HALO + r0 - DIL * w, rc), :] for w in range(W)]
                acc = ((p[0] + p[1]) + (p[2] + p[3])) + ((p[4] + p[5]) + (p[6] + p[7]))
                ot = (acc * rinv).astype(BF16)
                if t < 4:
                    o_s[jo, pl.ds(r0, rc), t * 128:(t + 1) * 128] = ot
                else:
                    o_s[jo, pl.ds(r0, rc), 512:576] = ot[:, 0:64]

        if kind == "o":
            for c in range(n):
                r0 = c * rc
                q = [q_s[j, t, pl.ds(r0, rc), :] for t in range(5)]
                T = []
                for w in range(W):
                    acc = logits(r0, w, q)
                    acc = acc + pltpu.roll(acc, 64, 1)
                    T.append(acc + pltpu.roll(acc, 32, 1))
                finish(r0, T)
        else:
            for c in range(n):
                r0 = c * rc
                q = [q_s[j, t, pl.ds(r0, rc), :] for t in range(5)]
                T = [logits(r0, w, q) for w in range(W)]
                T = [a + pltpu.roll(a, 64, 1) for a in T]
                T = [a + pltpu.roll(a, 32, 1) for a in T]
                finish(r0, T)

    state = {}

    def C_mxu(j):
        return _dg(wopT[...], o_s[j], NT)

    def C_ln(j, at):
        x1s = []
        for cidx in range(TM // 128):
            cols = pl.ds(cidx * 128, 128)
            x1 = xb[j, :, cols].astype(F32) + modT[pl.ds(2 * D, D), :] * at[:, cidx * 128:(cidx + 1) * 128]
            h2N[j, pl.ds(cidx * 128, 128), :] = ln_mod(x1, 3 * D, 4 * D).astype(BF16).T
            x1s.append(x1)
        return x1s

    def ffn_chunk(j, f, rows=None):
        hh = h2N[j] if rows is None else h2N[j, rows, :]
        a = jnp.maximum(_dg(hh, w1_v[:, f * FC:(f + 1) * FC], NN), 0.0).astype(BF16)
        return _dg(w2T_v[:, f * FC:(f + 1) * FC], a, NT)

    def acc_add(acc, y):
        gb = modT[pl.ds(5 * D, D), :]
        return [acc[c] + gb * y[:, c * 128:(c + 1) * 128] for c in range(len(acc))]

    def Dc(j, f, nsplit=1):
        if f < NF - 1 or nsplit == 1:
            state[("acc", j)] = acc_add(state[("acc", j)], ffn_chunk(j, f))
            if f == NF - 1:
                acc = state.pop(("acc", j))
                for c in range(TM // 128):
                    outb[j, :, pl.ds(c * 128, 128)] = acc[c].astype(BF16)
            return
        acc = state.pop(("acc", j))
        nt = TM // 128 // nsplit
        for sp in range(nsplit):
            part = acc_add(acc[sp * nt:(sp + 1) * nt], ffn_chunk(j, f, pl.ds(sp * nt * 128, nt * 128)))
            for c in range(nt):
                outb[j, :, pl.ds((sp * nt + c) * 128, 128)] = part[c].astype(BF16)
            out_copy(j, sp * nt * 128, nt * 128, 16 + sp).start()

    for ch in ORDER:
        if ch in "GHIJK":
            for d_ in gdm["GHIJK".index(ch)]:
                d_.start()
        else:
            dms[ch].start()
    zero_halo = jnp.zeros((HALO, 128), F32)
    for t in range(5):
        k_s[0, t, pl.ds(0, HALO), :] = zero_halo
        v_s[0, t, pl.ds(0, HALO), :] = zero_halo
    for i_st, st in enumerate(PROG.split()):
        k = st[0]
        if k == "L":
            ln1(int(st[1]))
        elif k == "S":
            stats0()
        elif k == "g":
            group0(int(st[1]))
        elif k == "K":
            for ch in st[3:]:
                A0k(int(st[1]), int(ch))
        elif k == "A":
            gs = range(4) if len(st) == 2 else [int(ch) for ch in st[3:]]
            for g in gs:
                A(int(st[1]), g)
        elif k == "B":
            B(int(st[1]), int(st[1]), st[3:], st[1] == "0")
        elif k == "C":
            jj = int(st[1])
            state[("acc", jj)] = C_ln(jj, C_mxu(jj))
        elif k == "c":
            state[("at", int(st[1]))] = C_mxu(int(st[1]))
        elif k == "l":
            jj = int(st[1])
            state[("acc", jj)] = C_ln(jj, state.pop(("at", jj)))
        elif k == "D":
            jj = int(st[1])
            lo, hi = (0, NF) if len(st) == 2 else map(int, st[3:].split("-"))
            for f in range(lo, hi):
                Dc(jj, f, LASTSPLIT if jj == NB - 1 else 1)
        elif k == "o":
            for ch in st[1:]:
                out_copy(int(ch), 0, TM, 13 + int(ch)).start()
        elif k == "|":
            pl.semaphore_signal(rsem, 1); pl.semaphore_wait(rsem, 1)
        elif k == "M":
            mod_part(2 * D, 4 * D); prep_wo()
        elif k == "w":
            with scope(f"s{i_st:02d}_{st[:2]}"):
                for ch in st[1:]:
                    if ch in "GHIJK":
                        for d_ in gdm["GHIJK".index(ch)]:
                            d_.wait()
                    else:
                        dms[ch].wait()

    with scope("z_wait_out"):
        for j in range(NB - 1):
            out_copy(j, 0, TM, 13 + j).wait()
        if LASTSPLIT == 1:
            out_copy(NB - 1, 0, TM, 13 + NB - 1).wait()
        for sp in range(LASTSPLIT if LASTSPLIT > 1 else 0):
            n = TM // LASTSPLIT
            out_copy(NB - 1, sp * n, n, 16 + sp).wait()


def _call(xT, wqkv, wo, w1, w2T, c, wm):
    hbm = pl.BlockSpec(memory_space=pltpu.HBM)
    scratch = [
        pltpu.VMEM((D, 3 * D), BF16),
        pltpu.VMEM((5, 3 * D, 128), F32),
        pltpu.VMEM((3 * D, D), BF16),
        pltpu.VMEM((D, D), BF16),
        pltpu.VMEM((5, D, 128), F32),
        pltpu.VMEM((D, D), BF16),
        pltpu.VMEM((D, FF), BF16),
        pltpu.VMEM((D, FF), BF16),
        pltpu.VMEM((D, 6 * D), BF16),
        pltpu.VMEM((1, D), BF16),
        pltpu.VMEM((6 * D, 128), F32),
        pltpu.VMEM((NB, D, TM), BF16),
        pltpu.VMEM((NB, TM, D), BF16),
        pltpu.VMEM((NB, 5, TM, 128), F32),
        pltpu.VMEM((NB, 5, HALO + TM, 128), F32),
        pltpu.VMEM((NB, 5, HALO + TM, 128), F32),
        pltpu.VMEM((NB, TM, D), BF16),
        pltpu.VMEM((NB, TM, D), BF16),
        pltpu.VMEM((NB, D, TM), BF16),
        pltpu.VMEM((192, TM), F32),
        pltpu.SemaphoreType.DMA((40,)),
        pltpu.SemaphoreType.REGULAR,
    ]
    return pl.pallas_call(
        kernel,
        out_shape=jax.ShapeDtypeStruct((D, S), BF16),
        in_specs=[hbm] * 7,
        out_specs=hbm,
        scratch_shapes=scratch,
        compiler_params=pltpu.CompilerParams(vmem_limit_bytes=110 * 1024 * 1024),
    )(xT, wqkv, wo, w1, w2T, c, wm)


@jax.jit
def pallas_adaLN_cond__sliding_local_dilated__dense_activation_relu__prompt_kernel(A_x, A_wqkv, A_wo, B_x, B_w1, B_w2, c, w_mod):
    xT = A_x.reshape(S, D).T
    outT = _call(xT, A_wqkv, A_wo, B_w1, B_w2.T, c, w_mod)
    return outT.T.reshape(1, S, D)
```

```python
import numpy as np
import jax
import jax.numpy as jnp
from jax import lax
import jax.experimental.pallas as pl
import jax.experimental.pallas.tpu as pltpu

S, D, H, DH, FF = 2048, 576, 32, 18, 4608
WIN, DIL = 8, 2
HALO = 16
TM = 512
NB = S // TM
LT = TM // 128
FC = 512
NF = FF // FC
RC = 8
EPS = 1e-5
F32, BF16 = jnp.float32, jnp.bfloat16
NN = (((1,), (0,)), ((), ()))
NT = (((1,), (1,)), ((), ()))
QSCALE = float(DH ** -0.5 * np.log2(np.e))

KGROUPS = ((512, 64), (0, 128), (128, 128), (256, 128), (384, 128))
MOD_TILES = ((4, 8), (0, 5), (1, 6), (2, 7), (3,))


def _dot(a, b, dims):
    return lax.dot_general(a, b, dims, preferred_element_type=F32)


def _dest_row(t, d):
    if d < 16:
        return t * 512 + d * H
    return 1536 + t * 64 + (d - 16) * H


def _tree(op, xs):
    while len(xs) > 1:
        xs = [op(xs[i], xs[i + 1]) for i in range(0, len(xs), 2)]
    return xs[0]


def _kernel(xT_hbm, wqkv_hbm, wo_hbm, w1_hbm, w2T_hbm, c_hbm, wm_hbm, outT_hbm,
            wqkv_v, wqkv_i, wpT, wo_v, wo32, wopT, w1_v, w2T_v, wm_v, c_v, sc_s, modT,
            xb, hN, q_s, k_s, v_s, tail_s, o_s, h2N, outb, dsem, bsem):
    sem_ids = iter(range(dsem.shape[0]))

    def copy(src, dst):
        return pltpu.make_async_copy(src, dst, dsem.at[next(sem_ids)])

    def wm_cols(lo, n):
        return copy(wm_hbm.at[:, pl.ds(lo, n)], wm_v.at[:, pl.ds(lo, n)])

    dm_x = [copy(xT_hbm.at[:, pl.ds(j * TM, TM)], xb.at[j]) for j in range(NB)]
    dm_c = copy(c_hbm, c_v)
    dm_g = [[copy(wqkv_hbm.at[pl.ds(r0, n), :], wqkv_v.at[pl.ds(r0, n), :])]
            + [wm_cols(t * 128, 128) for t in tiles]
            for (r0, n), tiles in zip(KGROUPS, MOD_TILES)]
    dm_wm = wm_cols(2 * D, 4 * D)
    dm_wo, dm_w1, dm_w2 = copy(wo_hbm, wo_v), copy(w1_hbm, w1_v), copy(w2T_hbm, w2T_v)
    dm_out = [copy(outb.at[j], outT_hbm.at[:, pl.ds(j * TM, TM)]) for j in range(NB - 1)]
    half = TM // 2
    dm_last = [copy(outb.at[NB - 1, :, pl.ds(i * half, half)],
                    outT_hbm.at[:, pl.ds((NB - 1) * TM + i * half, half)]) for i in range(2)]

    def wait(*ds):
        for d in ds:
            d.wait()

    def schedule_barrier():
        pl.semaphore_signal(bsem, 1)
        pl.semaphore_wait(bsem, 1)

    def silu_c():
        cf = c_v[...].astype(F32)
        sc_s[...] = jnp.broadcast_to((cf * jax.nn.sigmoid(cf)).astype(BF16), (16, D))

    def mod_part(lo, n):
        m = _dot(sc_s[...], wm_v[:, lo:lo + n], NN)[0:1, :]
        col = lo + lax.broadcasted_iota(jnp.int32, (1, n), 1)
        is_scale = ((col >= D) & (col < 2 * D)) | ((col >= 4 * D) & (col < 5 * D))
        m = m + jnp.where(is_scale, 1.0, 0.0)
        modT[pl.ds(lo, n), :] = jnp.broadcast_to(m, (128, n)).T

    def mod(i, r0=0, n=D):
        return modT[pl.ds(i * D + r0, n), :]

    def prep_wqkv_slab(s):
        n = min(128, D - 128 * s)
        wqkv_i[s, :, 0:n] = pltpu.bitcast(wqkv_v[pl.ds(128 * s, n), :].T, jnp.int32)
        for t in range(3):
            for d2 in range(DH // 2):
                words = wqkv_i[s, pl.ds(t * (D // 2) + d2, H, stride=DH // 2), :]
                lo = lax.bitcast_convert_type(words << 16, F32)
                hi = lax.bitcast_convert_type(words & jnp.int32(-65536), F32)
                for e, blk in enumerate((lo, hi)):
                    blk = (blk * QSCALE if t == 0 else blk).astype(BF16)
                    wpT[pl.ds(_dest_row(t, 2 * d2 + e), H), pl.ds(128 * s, n)] = blk[:, 0:n]

    def prep_wo():
        wof = wo_v[...].astype(F32)
        for s in range(4):
            wo32[s] = wof[:, s * 128:(s + 1) * 128]
        wo32[4] = jnp.concatenate([wof[:, 512:D], jnp.zeros((D, 64), F32)], axis=1)
        for s in range(5):
            blk = jnp.concatenate(
                [wo32[s, pl.ds(d, H, stride=DH), :] for d in range(DH)], axis=0)
            n = min(128, D - 128 * s)
            wopT[pl.ds(128 * s, n), :] = blk.T.astype(BF16)[0:n, :]

    def ln_stats(xf):
        mean = jnp.sum(xf, axis=0, keepdims=True) * (1.0 / D)
        xc = xf - mean
        var = jnp.sum(xc * xc, axis=0, keepdims=True) * (1.0 / D)
        return mean, xc, lax.rsqrt(var + EPS)

    def ln_mod(xf, shift, scale):
        _, xc, r = ln_stats(xf)
        return xc * r * mod(scale) + mod(shift)

    def x_tile(j, c, r0=0, n=D):
        return xb[j, pl.ds(r0, n), pl.ds(c * 128, 128)].astype(F32)

    def ln1(j):
        for c in range(LT):
            hN[j, pl.ds(c * 128, 128), :] = ln_mod(x_tile(j, c), 0, 1).astype(BF16).T

    def qkv_dot(g, h, k0, kn):
        if g < 3:
            return _dot(h, wpT[pl.ds(g * 512, 512), pl.ds(k0, kn)], NT)
        return _dot(wpT[pl.ds(1536, 192), pl.ds(k0, kn)], h, NT)

    def store_kv(dst, j, t, val):
        dst[j, t, pl.ds(HALO, TM), :] = val
        if j + 1 < NB:
            dst[j + 1, t, pl.ds(0, HALO), :] = val[TM - HALO:, :]

    def qkv_store(j, g, r):
        if g < 3:
            for t in range(4):
                val = r[:, t * 128:(t + 1) * 128]
                if g == 0:
                    q_s[j, t] = val
                else:
                    store_kv(k_s if g == 1 else v_s, j, t, val)
            return
        lo_half = lax.broadcasted_iota(jnp.int32, (TM, 128), 1) < 64
        qk, vt = r[0:128, :].T, r[128:192, :].T
        q_s[j, 4] = jnp.where(lo_half, qk, 0.0)
        store_kv(k_s, j, 4, jnp.where(lo_half, pltpu.roll(qk, 64, 1), 0.0))
        store_kv(v_s, j, 4, jnp.concatenate([vt, jnp.zeros_like(vt)], axis=1))

    def qkv(j, pieces):
        for g in pieces:
            qkv_store(j, g, qkv_dot(g, hN[j], 0, D))

    def block0_group(i, stats):
        for t in MOD_TILES[i]:
            mod_part(t * 128, 128)
        k0, kn = KGROUPS[i]
        prep_wqkv_slab(k0 // 128)
        for c, (mean, r) in enumerate(stats):
            h = (x_tile(0, c, k0, kn) - mean) * r * mod(1, k0, kn) + mod(0, k0, kn)
            hN[0, pl.ds(c * 128, 128), pl.ds(k0, kn)] = h.astype(BF16).T

    def block0_qkv(i, pieces):
        k0, kn = KGROUPS[i]
        first, last = i == 0, i == len(KGROUPS) - 1
        for g in pieces:
            r = qkv_dot(g, hN[0, :, pl.ds(k0, kn)], k0, kn)
            if g == 3:
                r = r if first else r + tail_s[...]
                if last:
                    qkv_store(0, 3, r)
                else:
                    tail_s[...] = r
                continue
            dst, rows = (q_s, k_s, v_s)[g], pl.ds(HALO if g else 0, TM)
            vals = [r[:, t * 128:(t + 1) * 128] for t in range(4)]
            if not first:
                vals = [v + dst[0, t, rows, :] for t, v in enumerate(vals)]
            if last:
                qkv_store(0, g, jnp.concatenate(vals, axis=1))
            else:
                for t in range(4):
                    dst[0, t, rows, :] = vals[t]

    def attention(j):
        for r0 in range(0, TM, RC):
            def win(ref, t, w):
                return ref[j, t, pl.ds(HALO + r0 - DIL * w, RC), :]

            q = [q_s[j, t, pl.ds(r0, RC), :] for t in range(5)]
            lg = []
            for w in range(WIN):
                p = [q[t] * win(k_s, t, w) for t in range(5)]
                lg.append(((p[0] + p[1]) + (p[2] + p[3])) + p[4])
            lg = [a + pltpu.roll(a, 64, 1) for a in lg]
            lg = [a + pltpu.roll(a, 32, 1) for a in lg]
            if j == 0 and r0 < HALO:
                pos = r0 + lax.broadcasted_iota(jnp.int32, (RC, 128), 0)
                lg = [jnp.where(pos >= DIL * w, a, -1e30) if w else a for w, a in enumerate(lg)]
            m = _tree(jnp.maximum, lg)
            e = [jnp.exp2(a - m) for a in lg]
            l = _tree(jnp.add, e)
            rinv = pl.reciprocal(l, approx=True)
            rinv = rinv * (2.0 - l * rinv)
            for t in range(5):
                ot = (_tree(jnp.add, [e[w] * win(v_s, t, w) for w in range(WIN)]) * rinv).astype(BF16)
                n = min(128, D - 128 * t)
                o_s[j, pl.ds(r0, RC), pl.ds(128 * t, n)] = ot[:, 0:n]

    def proj(j):
        at = _dot(wopT[...], o_s[j], NT)
        x1 = []
        for c in range(LT):
            x1.append(x_tile(j, c) + mod(2) * at[:, c * 128:(c + 1) * 128])
            h2N[j, pl.ds(c * 128, 128), :] = ln_mod(x1[c], 3, 4).astype(BF16).T
        return x1

    def mlp_chunk(j, f, acc, c0=0, nc=LT):
        cols = slice(f * FC, (f + 1) * FC)
        a = jnp.maximum(_dot(h2N[j, pl.ds(c0 * 128, nc * 128), :], w1_v[:, cols], NN), 0.0)
        y = _dot(w2T_v[:, cols], a.astype(BF16), NT)
        return [acc[c] + mod(5) * y[:, c * 128:(c + 1) * 128] for c in range(nc)]

    def mlp_head(j, acc):
        for f in range(NF - 1):
            acc = mlp_chunk(j, f, acc)
        return acc

    def mlp_tail(j, acc, c0=0, nc=LT):
        acc = mlp_chunk(j, NF - 1, acc[c0:c0 + nc], c0, nc)
        for c in range(nc):
            outb[j, :, pl.ds((c0 + c) * 128, 128)] = acc[c].astype(BF16)

    for d in (dm_x[0], dm_c, *dm_g[0], *dm_g[1], *dm_g[2], *dm_g[3], dm_x[1], *dm_g[4],
              dm_x[2], dm_x[3], dm_wm, dm_wo, dm_w1, dm_w2):
        d.start()
    wqkv_i[4] = jnp.zeros((3 * D // 2, 128), jnp.int32)
    for t in range(5):
        k_s[0, t, pl.ds(0, HALO), :] = jnp.zeros((HALO, 128), F32)
        v_s[0, t, pl.ds(0, HALO), :] = jnp.zeros((HALO, 128), F32)

    wait(dm_x[0])
    stats = [(mean, r) for mean, _, r in (ln_stats(x_tile(0, c)) for c in range(LT))]
    wait(dm_c, *dm_g[0])
    silu_c()
    block0_group(0, stats)
    block0_qkv(0, (3,))
    for i in range(1, len(KGROUPS)):
        wait(*dm_g[i], *((dm_x[1],) if i == len(KGROUPS) - 1 else ()))
        block0_group(i, stats)
        block0_qkv(i - 1, (0, 1, 2))
        if i < len(KGROUPS) - 1:
            block0_qkv(i, (3,))
    ln1(1)
    block0_qkv(len(KGROUPS) - 1, (3, 0, 1, 2))

    wait(dm_x[2], dm_x[3])
    qkv(1, (3, 0, 1, 2))
    ln1(2)

    wait(dm_wm, dm_wo)
    ln1(3)
    attention(0)
    qkv(2, (3, 0, 1, 2))
    mod_part(2 * D, 4 * D)
    prep_wo()
    qkv(3, (3, 0))

    wait(dm_w1)
    acc = proj(0)
    qkv(3, (1, 2))

    wait(dm_w2)
    acc = mlp_head(0, acc)
    for j in range(1, NB):
        attention(j)

    schedule_barrier()
    for j in range(1, NB):
        nxt = proj(j)
        mlp_tail(j - 1, acc)
        dm_out[j - 1].start()
        acc = mlp_head(j, nxt)
    for i in range(2):
        mlp_tail(NB - 1, acc, i * (LT // 2), LT // 2)
        dm_last[i].start()
    wait(*dm_out, *dm_last)


@jax.jit
def pallas_adaLN_cond__sliding_local_dilated__dense_activation_relu__prompt_kernel(
    A_x: jax.Array,
    A_wqkv: jax.Array,
    A_wo: jax.Array,
    B_x: jax.Array,
    B_w1: jax.Array,
    B_w2: jax.Array,
    c: jax.Array,
    w_mod: jax.Array,
):
    del B_x
    hbm = pl.BlockSpec(memory_space=pltpu.HBM)
    vmem = pltpu.VMEM
    n_dma = NB + 1 + len(KGROUPS) + sum(map(len, MOD_TILES)) + 4 + (NB - 1) + 2
    outT = pl.pallas_call(
        _kernel,
        out_shape=jax.ShapeDtypeStruct((D, S), BF16),
        in_specs=[hbm] * 7,
        out_specs=hbm,
        scratch_shapes=[
            vmem((D, 3 * D), BF16),
            vmem((5, 3 * D // 2, 128), jnp.int32),
            vmem((3 * D, D), BF16),
            vmem((D, D), BF16),
            vmem((5, D, 128), F32),
            vmem((D, D), BF16),
            vmem((D, FF), BF16),
            vmem((D, FF), BF16),
            vmem((D, 6 * D), BF16),
            vmem((1, D), BF16),
            vmem((16, D), BF16),
            vmem((6 * D, 128), F32),
            vmem((NB, D, TM), BF16),
            vmem((NB, TM, D), BF16),
            vmem((NB, 5, TM, 128), F32),
            vmem((NB, 5, HALO + TM, 128), F32),
            vmem((NB, 5, HALO + TM, 128), F32),
            vmem((192, TM), F32),
            vmem((NB, TM, D), BF16),
            vmem((NB, TM, D), BF16),
            vmem((NB, D, TM), BF16),
            pltpu.SemaphoreType.DMA((n_dma,)),
            pltpu.SemaphoreType.REGULAR,
        ],
        compiler_params=pltpu.CompilerParams(
            vmem_limit_bytes=110 * 1024 * 1024,
            flags={"XLA_TPU_EVENLY_DISTRIBUTE_CRITICAL_NODES": True},
        ),
    )(A_x.reshape(S, D).T, A_wqkv, A_wo, B_w1, B_w2.T, c, w_mod)
    return outT.T.reshape(1, S, D)
```

```python
import numpy as np
import jax
import jax.numpy as jnp
from jax import lax
import jax.experimental.pallas as pl
import jax.experimental.pallas.tpu as pltpu

S, D, H, DH, FF = 2048, 576, 32, 18, 4608
WIN, DIL = 8, 2
HALO = 16
TM = 512
NB = S // TM
LT = TM // 128
FC = 512
NF = FF // FC
RC = 8
EPS = 1e-5
F32, BF16 = jnp.float32, jnp.bfloat16
NN = (((1,), (0,)), ((), ()))
NT = (((1,), (1,)), ((), ()))
QSCALE = float(DH ** -0.5 * np.log2(np.e))

KGROUPS = ((512, 64), (0, 128), (128, 128), (256, 128), (384, 128))
MOD_TILES = ((4, 8), (0, 5), (1, 6), (2, 7), (3,))


def _dot(a, b, dims):
    return lax.dot_general(a, b, dims, preferred_element_type=F32)


def _dest_row(t, d):
    if d < 16:
        return t * 512 + d * H
    return 1536 + t * 64 + (d - 16) * H


def _tree(op, xs):
    while len(xs) > 1:
        xs = [op(xs[i], xs[i + 1]) for i in range(0, len(xs), 2)]
    return xs[0]


def _kernel(xT_hbm, wqkv_hbm, wo_hbm, w1_hbm, w2T_hbm, c_hbm, wm_hbm, outT_hbm,
            wqkv_v, wqkv_i, wpT, wo_v, wo_i, wopT, w1_v, w2T_v, wm_v, c_v, sc_s, modT,
            xb, hN, q_s, k_s, v_s, tail_s, o_s, h2N, outb, dsem, bsem):
    sem_ids = iter(range(dsem.shape[0]))

    def copy(src, dst):
        return pltpu.make_async_copy(src, dst, dsem.at[next(sem_ids)])

    def wm_cols(lo, n):
        return copy(wm_hbm.at[:, pl.ds(lo, n)], wm_v.at[:, pl.ds(lo, n)])

    dm_x = [copy(xT_hbm.at[:, pl.ds(j * TM, TM)], xb.at[j]) for j in range(NB)]
    dm_c = copy(c_hbm, c_v)
    dm_g = [[copy(wqkv_hbm.at[pl.ds(r0, n), :], wqkv_v.at[pl.ds(r0, n), :])]
            + [wm_cols(t * 128, 128) for t in tiles]
            for (r0, n), tiles in zip(KGROUPS, MOD_TILES)]
    dm_wm = wm_cols(2 * D, 4 * D)
    dm_wo, dm_w1, dm_w2 = copy(wo_hbm, wo_v), copy(w1_hbm, w1_v), copy(w2T_hbm, w2T_v)
    dm_out = [copy(outb.at[j], outT_hbm.at[:, pl.ds(j * TM, TM)]) for j in range(NB - 1)]
    half = TM // 2
    dm_last = [copy(outb.at[NB - 1, :, pl.ds(i * half, half)],
                    outT_hbm.at[:, pl.ds((NB - 1) * TM + i * half, half)]) for i in range(2)]

    def wait(*ds):
        for d in ds:
            d.wait()

    def schedule_barrier():
        pl.semaphore_signal(bsem, 1)
        pl.semaphore_wait(bsem, 1)

    def silu_c():
        cf = c_v[...].astype(F32)
        sc_s[...] = jnp.broadcast_to((cf * jax.nn.sigmoid(cf)).astype(BF16), (16, D))

    def mod_part(lo, n):
        m = _dot(sc_s[...], wm_v[:, lo:lo + n], NN)[0:1, :]
        col = lo + lax.broadcasted_iota(jnp.int32, (1, n), 1)
        is_scale = ((col >= D) & (col < 2 * D)) | ((col >= 4 * D) & (col < 5 * D))
        m = m + jnp.where(is_scale, 1.0, 0.0)
        modT[pl.ds(lo, n), :] = jnp.broadcast_to(m, (128, n)).T

    def mod(i, r0=0, n=D):
        return modT[pl.ds(i * D + r0, n), :]

    def prep_wqkv_slab(s):
        n = min(128, D - 128 * s)
        wqkv_i[s, :, 0:n] = pltpu.bitcast(wqkv_v[pl.ds(128 * s, n), :].T, jnp.int32)
        for t in range(3):
            for d2 in range(DH // 2):
                words = wqkv_i[s, pl.ds(t * (D // 2) + d2, H, stride=DH // 2), :]
                lo = lax.bitcast_convert_type(words << 16, F32)
                hi = lax.bitcast_convert_type(words & jnp.int32(-65536), F32)
                for e, blk in enumerate((lo, hi)):
                    blk = (blk * QSCALE if t == 0 else blk).astype(BF16)
                    wpT[pl.ds(_dest_row(t, 2 * d2 + e), H), pl.ds(128 * s, n)] = blk[:, 0:n]

    def prep_wo():
        words = pltpu.bitcast(wo_v[...], jnp.int32)
        for s in range(4):
            wo_i[s] = words[:, s * 128:(s + 1) * 128]
        wo_i[4] = jnp.concatenate([words[:, 512:D], jnp.zeros((D // 2, 64), jnp.int32)], axis=1)
        for s in range(5):
            rows = []
            for d2 in range(DH // 2):
                w = wo_i[s, pl.ds(d2, H, stride=DH // 2), :]
                rows.append(lax.bitcast_convert_type(w << 16, F32).astype(BF16))
                rows.append(lax.bitcast_convert_type(w & jnp.int32(-65536), F32).astype(BF16))
            n = min(128, D - 128 * s)
            wopT[pl.ds(128 * s, n), :] = jnp.concatenate(rows, axis=0).T[0:n, :]

    def ln_stats(xf):
        mean = jnp.sum(xf, axis=0, keepdims=True) * (1.0 / D)
        xc = xf - mean
        var = jnp.sum(xc * xc, axis=0, keepdims=True) * (1.0 / D)
        return mean, xc, lax.rsqrt(var + EPS)

    def ln_mod(xf, shift, scale):
        _, xc, r = ln_stats(xf)
        return xc * r * mod(scale) + mod(shift)

    def x_tile(j, c, r0=0, n=D):
        return xb[j, pl.ds(r0, n), pl.ds(c * 128, 128)].astype(F32)

    def ln1(j):
        for c in range(LT):
            hN[j, pl.ds(c * 128, 128), :] = ln_mod(x_tile(j, c), 0, 1).astype(BF16).T

    def qkv_dot(g, h, k0, kn):
        if g < 3:
            return _dot(h, wpT[pl.ds(g * 512, 512), pl.ds(k0, kn)], NT)
        return _dot(wpT[pl.ds(1536, 192), pl.ds(k0, kn)], h, NT)

    def store_kv(dst, j, t, val):
        dst[j, t, pl.ds(HALO, TM), :] = val
        if j + 1 < NB:
            dst[j + 1, t, pl.ds(0, HALO), :] = val[TM - HALO:, :]

    def qkv_store(j, g, r):
        if g < 3:
            for t in range(4):
                val = r[:, t * 128:(t + 1) * 128]
                if g == 0:
                    q_s[j, t] = val
                else:
                    store_kv(k_s if g == 1 else v_s, j, t, val)
            return
        lo_half = lax.broadcasted_iota(jnp.int32, (TM, 128), 1) < 64
        qk, vt = r[0:128, :].T, r[128:192, :].T
        q_s[j, 4] = jnp.where(lo_half, qk, 0.0)
        store_kv(k_s, j, 4, jnp.where(lo_half, pltpu.roll(qk, 64, 1), 0.0))
        store_kv(v_s, j, 4, jnp.concatenate([vt, jnp.zeros_like(vt)], axis=1))

    def qkv(j, pieces):
        for g in pieces:
            qkv_store(j, g, qkv_dot(g, hN[j], 0, D))

    def block0_group(i, stats):
        for t in MOD_TILES[i]:
            mod_part(t * 128, 128)
        k0, kn = KGROUPS[i]
        prep_wqkv_slab(k0 // 128)
        for c, (mean, r) in enumerate(stats):
            h = (x_tile(0, c, k0, kn) - mean) * r * mod(1, k0, kn) + mod(0, k0, kn)
            hN[0, pl.ds(c * 128, 128), pl.ds(k0, kn)] = h.astype(BF16).T

    def block0_qkv(i, pieces):
        k0, kn = KGROUPS[i]
        first, last = i == 0, i == len(KGROUPS) - 1
        for g in pieces:
            r = qkv_dot(g, hN[0, :, pl.ds(k0, kn)], k0, kn)
            if g == 3:
                r = r if first else r + tail_s[...]
                if last:
                    qkv_store(0, 3, r)
                else:
                    tail_s[...] = r
                continue
            dst, rows = (q_s, k_s, v_s)[g], pl.ds(HALO if g else 0, TM)
            vals = [r[:, t * 128:(t + 1) * 128] for t in range(4)]
            if not first:
                vals = [v + dst[0, t, rows, :] for t, v in enumerate(vals)]
            if last:
                qkv_store(0, g, jnp.concatenate(vals, axis=1))
            else:
                for t in range(4):
                    dst[0, t, rows, :] = vals[t]

    def attention(j):
        for r0 in range(0, TM, RC):
            def win(ref, t, w):
                return ref[j, t, pl.ds(HALO + r0 - DIL * w, RC), :]

            q = [q_s[j, t, pl.ds(r0, RC), :] for t in range(5)]
            lg = []
            for w in range(WIN):
                p = [q[t] * win(k_s, t, w) for t in range(5)]
                lg.append(((p[0] + p[1]) + (p[2] + p[3])) + p[4])
            lg = [a + pltpu.roll(a, 64, 1) for a in lg]
            lg = [a + pltpu.roll(a, 32, 1) for a in lg]
            if j == 0 and r0 < HALO:
                pos = r0 + lax.broadcasted_iota(jnp.int32, (RC, 128), 0)
                lg = [jnp.where(pos >= DIL * w, a, -1e30) if w else a for w, a in enumerate(lg)]
            m = _tree(jnp.maximum, lg)
            e = [jnp.exp2(a - m) for a in lg]
            l = _tree(jnp.add, e)
            rinv = pl.reciprocal(l, approx=True)
            rinv = rinv * (2.0 - l * rinv)
            for t in range(5):
                ot = (_tree(jnp.add, [e[w] * win(v_s, t, w) for w in range(WIN)]) * rinv).astype(BF16)
                n = min(128, D - 128 * t)
                o_s[j, pl.ds(r0, RC), pl.ds(128 * t, n)] = ot[:, 0:n]

    def proj(j):
        at = _dot(wopT[...], o_s[j], NT)
        x1 = []
        for c in range(LT):
            x1.append(x_tile(j, c) + mod(2) * at[:, c * 128:(c + 1) * 128])
            h2N[j, pl.ds(c * 128, 128), :] = ln_mod(x1[c], 3, 4).astype(BF16).T
        return x1

    def mlp_chunk(j, f, acc, c0=0, nc=LT):
        cols = slice(f * FC, (f + 1) * FC)
        a = jnp.maximum(_dot(h2N[j, pl.ds(c0 * 128, nc * 128), :], w1_v[:, cols], NN), 0.0)
        y = _dot(w2T_v[:, cols], a.astype(BF16), NT)
        return [acc[c] + mod(5) * y[:, c * 128:(c + 1) * 128] for c in range(nc)]

    def mlp_head(j, acc):
        for f in range(NF - 1):
            acc = mlp_chunk(j, f, acc)
        return acc

    def mlp_tail(j, acc, c0=0, nc=LT):
        acc = mlp_chunk(j, NF - 1, acc[c0:c0 + nc], c0, nc)
        for c in range(nc):
            outb[j, :, pl.ds((c0 + c) * 128, 128)] = acc[c].astype(BF16)

    for d in (dm_x[0], dm_c, *dm_g[0], *dm_g[1], *dm_g[2], *dm_g[3], dm_x[1], *dm_g[4],
              dm_x[2], dm_x[3], dm_wm, dm_wo, dm_w1, dm_w2):
        d.start()
    wqkv_i[4] = jnp.zeros((3 * D // 2, 128), jnp.int32)
    for t in range(5):
        k_s[0, t, pl.ds(0, HALO), :] = jnp.zeros((HALO, 128), F32)
        v_s[0, t, pl.ds(0, HALO), :] = jnp.zeros((HALO, 128), F32)

    wait(dm_x[0])
    stats = [(mean, r) for mean, _, r in (ln_stats(x_tile(0, c)) for c in range(LT))]
    wait(dm_c, *dm_g[0])
    silu_c()
    block0_group(0, stats)
    block0_qkv(0, (3,))
    for i in range(1, len(KGROUPS)):
        wait(*dm_g[i], *((dm_x[1],) if i == len(KGROUPS) - 1 else ()))
        block0_group(i, stats)
        block0_qkv(i - 1, (0, 1, 2))
        if i < len(KGROUPS) - 1:
            block0_qkv(i, (3,))
    ln1(1)
    block0_qkv(len(KGROUPS) - 1, (3, 0, 1, 2))

    wait(dm_x[2], dm_x[3])
    qkv(1, (3, 0, 1, 2))
    ln1(2)

    wait(dm_wm, dm_wo)
    ln1(3)
    attention(0)
    qkv(2, (3, 0, 1, 2))
    mod_part(2 * D, 4 * D)
    prep_wo()
    qkv(3, (3, 0))

    wait(dm_w1)
    acc = proj(0)
    qkv(3, (1, 2))

    wait(dm_w2)
    acc = mlp_head(0, acc)
    for j in range(1, NB):
        attention(j)

    schedule_barrier()
    for j in range(1, NB):
        nxt = proj(j)
        mlp_tail(j - 1, acc)
        dm_out[j - 1].start()
        acc = mlp_head(j, nxt)
    for i in range(2):
        mlp_tail(NB - 1, acc, i * (LT // 2), LT // 2)
        dm_last[i].start()
    wait(*dm_out, *dm_last)


@jax.jit
def pallas_adaLN_cond__sliding_local_dilated__dense_activation_relu__prompt_kernel(
    A_x: jax.Array,
    A_wqkv: jax.Array,
    A_wo: jax.Array,
    B_x: jax.Array,
    B_w1: jax.Array,
    B_w2: jax.Array,
    c: jax.Array,
    w_mod: jax.Array,
):
    del B_x
    hbm = pl.BlockSpec(memory_space=pltpu.HBM)
    vmem = pltpu.VMEM
    n_dma = NB + 1 + len(KGROUPS) + sum(map(len, MOD_TILES)) + 4 + (NB - 1) + 2
    outT = pl.pallas_call(
        _kernel,
        out_shape=jax.ShapeDtypeStruct((D, S), BF16),
        in_specs=[hbm] * 7,
        out_specs=hbm,
        scratch_shapes=[
            vmem((D, 3 * D), BF16),
            vmem((5, 3 * D // 2, 128), jnp.int32),
            vmem((3 * D, D), BF16),
            vmem((D, D), BF16),
            vmem((5, D // 2, 128), jnp.int32),
            vmem((D, D), BF16),
            vmem((D, FF), BF16),
            vmem((D, FF), BF16),
            vmem((D, 6 * D), BF16),
            vmem((1, D), BF16),
            vmem((16, D), BF16),
            vmem((6 * D, 128), F32),
            vmem((NB, D, TM), BF16),
            vmem((NB, TM, D), BF16),
            vmem((NB, 5, TM, 128), F32),
            vmem((NB, 5, HALO + TM, 128), F32),
            vmem((NB, 5, HALO + TM, 128), F32),
            vmem((192, TM), F32),
            vmem((NB, TM, D), BF16),
            vmem((NB, TM, D), BF16),
            vmem((NB, D, TM), BF16),
            pltpu.SemaphoreType.DMA((n_dma,)),
            pltpu.SemaphoreType.REGULAR,
        ],
        compiler_params=pltpu.CompilerParams(
            vmem_limit_bytes=110 * 1024 * 1024,
            flags={"XLA_TPU_EVENLY_DISTRIBUTE_CRITICAL_NODES": True},
        ),
    )(A_x.reshape(S, D).T, A_wqkv, A_wo, B_w1, B_w2.T, c, w_mod)
    return outT.T.reshape(1, S, D)
```
